```python
import os as _os
_os.environ.setdefault("JAX_PLATFORMS", "cpu")
import jax
import jax.numpy as jnp

def _softmax(x, axis=-1):
    return jax.nn.softmax(x, axis=axis)
def _gelu(x):
    return jax.nn.gelu(x, approximate=True)
def _silu(x):
    return jax.nn.silu(x)
def _sigmoid(x):
    return jax.nn.sigmoid(x)
def _layernorm(x, axis=-1, eps=1e-5):
    m = jnp.mean(x, axis=axis, keepdims=True)
    v = jnp.var(x, axis=axis, keepdims=True)
    return (x - m) / jnp.sqrt(v + eps)
def _scatter_add(tgt, idx, src, axis=0):
    return tgt.at[idx].add(src)
def _segment_sum(src, seg, n):
    return jax.ops.segment_sum(src, seg, n)
class _Rng:
    def __init__(self, key):
        self._k = key
    def _next(self):
        self._k, sub = jax.random.split(self._k)
        return sub
    def normal(self, shape):
        return jax.random.normal(self._next(), shape, dtype=jnp.bfloat16)
    def randint(self, lo, hi, shape):
        return jax.random.randint(self._next(), shape, lo, hi, dtype=jnp.int32)
    def uniform(self, shape, lo=0.0, hi=1.0):
        return jax.random.uniform(self._next(), shape, jnp.bfloat16, lo, hi)
    def permutation(self, n):
        return jax.random.permutation(self._next(), n)


kernel_name = 'standalone__linear_kernel_rfa__decode'

def setup_inputs():
    _rng = _Rng(jax.random.key(int.from_bytes(__import__("os").urandom(4), "little")))
    _w = (lambda a: (lambda t: t.astype(jnp.bfloat16) if jnp.issubdtype(t.dtype, jnp.floating) else t)(jnp.asarray(a)))
    B, H, Sq, Sk, D, M = 2, 16, 1, 16384, 256, 16
    return {
        "q": _w((lambda *s: _rng.normal(s) * 0.4)(B, H, Sq, D)),
        "k": _w((lambda *s: _rng.normal(s) * 1.6)(B, H, Sk, D)),
        "v": _w((lambda *s: _rng.normal(s) * 1.6)(B, H, Sk, D)),
        "omega": _w((lambda *s: _rng.normal(s) * 1.6)(M, D)),
    }

def reference(q, k, v, omega):
    d = q.shape[-1]
    m = omega.shape[0]
    scale = float(d) ** -0.25
    qs = q * scale
    ks = k * scale
    q_proj = jnp.einsum("bhsd,md->bhsm", qs, omega)
    k_proj = jnp.einsum("bhsd,md->bhsm", ks, omega)
    q_sq = 0.5 * jnp.einsum("bhsd,bhsd->bhs", qs, qs)[..., None]
    k_sq = 0.5 * jnp.einsum("bhsd,bhsd->bhs", ks, ks)[..., None]
    inv_sqrt_m = float(m) ** -0.5
    phi_q = jnp.exp(q_proj - q_sq) * inv_sqrt_m + 1e-6
    phi_k = jnp.exp(k_proj - k_sq) * inv_sqrt_m + 1e-6
    kv = jnp.einsum("bhsm,bhsd->bhmd", phi_k, v)
    z  = jnp.einsum("bhsm->bhm", phi_k)
    num = jnp.einsum("bhqm,bhmd->bhqd", phi_q, kv)
    den = jnp.einsum("bhqm,bhm->bhq", phi_q, z)[..., None] + 1e-6
    return num / den
```

```python
import functools
import jax
import jax.numpy as jnp
import jax.experimental.pallas as pl
import jax.experimental.pallas.tpu as pltpu

TS = 1024
CH = 1024
_NT = (((1,), (1,)), ((), ()))


def _kernel(q_ref, k_ref, v_ref, om_ref, o_ref, kv_ref, z_ref, *, ts, ch):
    j = pl.program_id(1)
    d = k_ref.shape[-1]
    m = om_ref.shape[0]
    h = d // 2
    scale = float(d) ** -0.25
    inv_sqrt_m = float(m) ** -0.5

    @pl.when(j == 0)
    def _():
        kv_ref[...] = jnp.zeros_like(kv_ref)
        z_ref[...] = jnp.zeros_like(z_ref)

    om = om_ref[...]
    ones = jnp.ones((m, h), jnp.bfloat16)
    kv = kv_ref[...]
    z = z_ref[...]
    for c in range(ts // ch):
        k = k_ref[pl.ds(c * ch, ch), :]
        v = v_ref[pl.ds(c * ch, ch), :]
        proj = jax.lax.dot_general(om, k, _NT, preferred_element_type=jnp.float32)
        kf = k.astype(jnp.float32)
        a, b = kf[:, :h], kf[:, h:]
        k2 = (a * a + b * b).astype(jnp.bfloat16)
        sq = jax.lax.dot_general(ones, k2, _NT, preferred_element_type=jnp.float32)
        phi = jnp.exp(proj * scale - sq * (0.5 * scale * scale)) * inv_sqrt_m + 1e-6
        pb = phi.astype(jnp.bfloat16)
        kv = kv + jnp.dot(pb, v, preferred_element_type=jnp.float32)
        pf = pb.astype(jnp.float32)
        for t in range(ch // 128):
            z = z + pf[:, t * 128:(t + 1) * 128]
    kv_ref[...] = kv
    z_ref[...] = z

    @pl.when(j == pl.num_programs(1) - 1)
    def _():
        qs = q_ref[...].astype(jnp.float32) * scale
        qp = jnp.sum(om.astype(jnp.float32) * qs, axis=1, keepdims=True)
        qsq = 0.5 * jnp.sum(qs * qs, axis=1, keepdims=True)
        pq = jnp.exp(qp - qsq) * inv_sqrt_m + 1e-6
        num = jnp.sum(pq * kv, axis=0, keepdims=True)
        zz = jnp.sum(z, axis=1, keepdims=True)
        den = jnp.sum(pq * zz, axis=0, keepdims=True) + 1e-6
        o_ref[...] = (num / den).astype(o_ref.dtype)


@jax.jit
def pallas_standalone__linear_kernel_rfa__decode_kernel(q, k, v, omega):
    B, H, Sq, D = q.shape
    Sk = k.shape[2]
    M = omega.shape[0]
    assert Sq == 1
    ts = min(TS, Sk)
    ch = min(CH, ts)
    assert Sk % ts == 0 and ts % ch == 0 and ch % 128 == 0
    G = B * H
    out = pl.pallas_call(
        functools.partial(_kernel, ts=ts, ch=ch),
        grid=(G, Sk // ts),
        in_specs=[
            pl.BlockSpec((None, 1, D), lambda g, j: (g, 0, 0)),
            pl.BlockSpec((None, ts, D), lambda g, j: (g, j, 0)),
            pl.BlockSpec((None, ts, D), lambda g, j: (g, j, 0)),
            pl.BlockSpec((M, D), lambda g, j: (0, 0)),
        ],
        out_specs=pl.BlockSpec((None, 1, D), lambda g, j: (g, 0, 0)),
        out_shape=jax.ShapeDtypeStruct((G, 1, D), q.dtype),
        scratch_shapes=[pltpu.VMEM((M, D), jnp.float32),
                        pltpu.VMEM((M, 128), jnp.float32)],
        compiler_params=pltpu.CompilerParams(
            dimension_semantics=("parallel", "arbitrary"),
            vmem_limit_bytes=64 * 1024 * 1024),
    )(q.reshape(G, 1, D), k.reshape(G, Sk, D), v.reshape(G, Sk, D), omega)
    return out.reshape(B, H, 1, D)
```
